```python
import os as _os
_os.environ.setdefault("JAX_PLATFORMS", "cpu")
import jax
import jax.numpy as jnp

def _softmax(x, axis=-1):
    return jax.nn.softmax(x, axis=axis)
def _gelu(x):
    return jax.nn.gelu(x, approximate=True)
def _silu(x):
    return jax.nn.silu(x)
def _sigmoid(x):
    return jax.nn.sigmoid(x)
def _layernorm(x, axis=-1, eps=1e-5):
    m = jnp.mean(x, axis=axis, keepdims=True)
    v = jnp.var(x, axis=axis, keepdims=True)
    return (x - m) / jnp.sqrt(v + eps)
def _scatter_add(tgt, idx, src, axis=0):
    return tgt.at[idx].add(src)
def _segment_sum(src, seg, n):
    return jax.ops.segment_sum(src, seg, n)
class _Rng:
    def __init__(self, key):
        self._k = key
    def _next(self):
        self._k, sub = jax.random.split(self._k)
        return sub
    def normal(self, shape):
        return jax.random.normal(self._next(), shape, dtype=jnp.bfloat16)
    def randint(self, lo, hi, shape):
        return jax.random.randint(self._next(), shape, lo, hi, dtype=jnp.int32)
    def uniform(self, shape, lo=0.0, hi=1.0):
        return jax.random.uniform(self._next(), shape, jnp.bfloat16, lo, hi)
    def permutation(self, n):
        return jax.random.permutation(self._next(), n)


kernel_name = 'gated_mix__mha_block__mixer_s_mlp__prompt'

def setup_inputs():
    _rng = _Rng(jax.random.key(int.from_bytes(__import__("os").urandom(4), "little")))
    _w = (lambda a: (lambda t: t.astype(jnp.bfloat16) if jnp.issubdtype(t.dtype, jnp.floating) else t)(jnp.asarray(a)))
    def _A_setup():
        B, S, D, H = 1, 2048, 448, 16
        return {
            "x": _w((lambda *s: _rng.normal(s) * 0.05)(B, S, D)),
            "wqkv": _w((lambda *s: _rng.normal(s) * 0.8)(D, 3 * D)),
            "wo": _w((lambda *s: _rng.normal(s) * 0.05)(D, D)),
        }
    _A_in = _A_setup()

    def _B_setup():
        B, S, D, F = 1, 2048, 448, 1792
        return {
            "x":  _w((lambda *s: _rng.normal(s) * 0.05)(B, S, D)),
            "w1": _w((lambda *s: _rng.normal(s) * 0.2)(D, D) * (D ** -0.5)),
            "w2": _w((lambda *s: _rng.normal(s) * 0.2)(D, D) * (D ** -0.5)),
            "w3": _w((lambda *s: _rng.normal(s) * 0.2)(D, F) * (D ** -0.5)),
            "w4": _w((lambda *s: _rng.normal(s) * 0.2)(F, D) * (F ** -0.5)),
        }
    _B_in = _B_setup()

    return {
        "A_x": _A_in["x"],
        "A_wqkv": _A_in["wqkv"],
        "A_wo": _A_in["wo"],
        "B_x": _B_in["x"],
        "B_w1": _B_in["w1"],
        "B_w2": _B_in["w2"],
        "B_w3": _B_in["w3"],
        "B_w4": _B_in["w4"],
        "gate_w": _w((lambda *s: _rng.normal(s) * 0.05)(448) * 16.0),
    }

def reference(A_x, A_wqkv, A_wo, B_x, B_w1, B_w2, B_w3, B_w4, gate_w):
    def _A_ref(x, wqkv, wo):
        B, S, D = x.shape
        H = 16
        Dh = D // H
        qkv = (lambda x, *d: x.transpose(*d))((x @ wqkv).reshape(B, S, 3, H, Dh), 2, 0, 3, 1, 4)
        q, k, v = qkv[0], qkv[1], qkv[2]
        scores = jnp.einsum("bhqd,bhkd->bhqk", q, k) * (Dh ** -0.5)
        p = _softmax(scores, axis=-1)
        o = jnp.einsum("bhqk,bhkd->bhqd", p, v)
        return (lambda x, *d: x.transpose(*d))(o, 0, 2, 1, 3).reshape(B, S, D) @ wo

    def _B_ref(x, w1, w2, w3, w4):
        B, S, D = x.shape
        h = _gelu(_layernorm(x, axis=-1) @ w1)
        c = D // 4
        g0 = jnp.pad(h[:, :, 0*c:1*c], ((0, 0), (1, 0), (0, 0)))[:, :S, :]
        g1 = jnp.pad(h[:, :, 1*c:2*c], ((0, 0), (0, 1), (0, 0)))[:, 1:, :]
        g2 = jnp.pad(h[:, :, 2*c:3*c], ((0, 0), (2, 0), (0, 0)))[:, :S, :]
        g3 = jnp.pad(h[:, :, 3*c:   ], ((0, 0), (0, 2), (0, 0)))[:, 2:, :]
        hs = jnp.concatenate([g0, g1, g2, g3], axis=-1) @ w2
        x1 = x + hs
        h2 = _gelu(_layernorm(x1, axis=-1) @ w3) @ w4
        return x1 + h2

    x = A_x
    g = _sigmoid((x * gate_w).sum(-1, keepdims=True))
    a = _A_ref(x, A_wqkv, A_wo)
    b = _B_ref(x, B_w1, B_w2, B_w3, B_w4)
    return g * a + (1 - g) * b
```

```python
import functools
import math

import jax
import jax.numpy as jnp
import jax.experimental.pallas as pl
import jax.experimental.pallas.tpu as pltpu

T = 2048
D = 448
H = 16
DH = 28
F = 1792
G = 112
HP = 32
TQ = 512
CK = 256
TP = 512
HALO = 128
EPS = 1e-5
QSCALE = (DH ** -0.5) * math.log2(math.e)
GROW = 3 * D

f32 = jnp.float32
bf16 = jnp.bfloat16


def _gelu(x):
    c = math.sqrt(2.0 / math.pi)
    inner = x * (c + (c * 0.044715) * (x * x))
    hx = 0.5 * x
    return hx + hx * jnp.tanh(inner)


def _layernorm_t(x):
    m = jnp.sum(x, axis=0, keepdims=True) * (1.0 / D)
    xc = x - m
    v = jnp.sum(xc * xc, axis=0, keepdims=True) * (1.0 / D)
    return xc * jax.lax.rsqrt(v + EPS)


def _dot(a, b):
    return jnp.dot(a, b, preferred_element_type=f32)


def _kernel(xt_hbm, wqkv_hbm, wo_hbm, w1_hbm, w2_hbm, w3_hbm, w4t_hbm, gw_ref,
            out_ref,
            xt_s, wqkv_v, wo_v, w1_v, w2_v, w3_v, w4t_s, sems,
            wqkvT_s, w1T_s, w2T_s, w3T_s, woT_s,
            k_s, qp_s, vt_s, ht_s, g_s, tmp_s,
            sa, sb, ma, mb, ot_s):
    step = pl.program_id(0)
    NC = T // CK

    @pl.when(step == 0)
    def _prologue():
        cp_wqkv = pltpu.make_async_copy(wqkv_hbm, wqkv_v, sems.at[0])
        cp_w1 = pltpu.make_async_copy(w1_hbm, w1_v, sems.at[1])
        cp_x0 = pltpu.make_async_copy(xt_hbm.at[:, 0:TP], xt_s.at[:, 0:TP], sems.at[2])
        cp_x1 = pltpu.make_async_copy(xt_hbm.at[:, TP:], xt_s.at[:, TP:], sems.at[3])
        cp_w3 = pltpu.make_async_copy(w3_hbm, w3_v, sems.at[4])
        cp_w2 = pltpu.make_async_copy(w2_hbm, w2_v, sems.at[5])
        cp_wo = pltpu.make_async_copy(wo_hbm, wo_v, sems.at[6])
        cp_w4 = pltpu.make_async_copy(w4t_hbm, w4t_s, sems.at[7])
        cp_wqkv.start()
        cp_w1.start()
        cp_x0.start()
        ht_s[:, 0:HALO] = jnp.zeros((D, HALO), bf16)
        ht_s[:, HALO + T:] = jnp.zeros((D, HALO), bf16)
        row16 = jax.lax.broadcasted_iota(jnp.int32, (16, D), 0)
        gw = jnp.broadcast_to(gw_ref[...].astype(f32).reshape(1, D), (16, D))
        wqkvT_s[GROW:GROW + 16, :] = jnp.where(row16 == 0, gw, 0.0).astype(bf16)
        cp_wqkv.wait()
        cp_x1.start()
        cp_w3.start()
        cp_w2.start()
        cp_wo.start()
        cp_w4.start()
        wqkvT_s[0:GROW, :] = wqkv_v[...].T
        cp_w1.wait()
        w1T_s[...] = w1_v[...].T
        cp_x0.wait()

        row_g = jax.lax.broadcasted_iota(jnp.int32, (G, TP), 0)
        row_h = jax.lax.broadcasted_iota(jnp.int32, (HP, TP), 0)

        for c in range(T // TP):
            t0 = c * TP
            if c == 1:
                cp_x1.wait()
                cp_w3.wait()
                cp_w2.wait()
                cp_wo.wait()
                cp_w4.wait()
            xc = xt_s[:, t0:t0 + TP]
            r = _dot(wqkvT_s[...], xc)
            for g in range(4):
                qg = r[g * G:(g + 1) * G, :] * QSCALE
                for j in range(4):
                    msk = (row_g >= j * DH) & (row_g < (j + 1) * DH)
                    qp_s[4 * g + j, :, t0:t0 + TP] = jnp.where(msk, qg, 0.0).astype(bf16)
                k_s[g, t0:t0 + TP, :] = r[D + g * G:D + (g + 1) * G, :].astype(bf16).T
            tmp_s[...] = r[2 * D:3 * D + 8, :]
            for h in range(H):
                vh = tmp_s[h * DH:h * DH + HP, :]
                vh = jnp.where(row_h < DH, vh, jnp.where(row_h == DH, 1.0, 0.0))
                vt_s[h, :, t0:t0 + TP] = vh.astype(bf16)
            g_s[:, t0:t0 + TP] = jax.nn.sigmoid(r[GROW:GROW + 1, :])
            xn = _layernorm_t(xc.astype(f32)).astype(bf16)
            ht_s[:, HALO + t0:HALO + t0 + TP] = _gelu(_dot(w1T_s[...], xn)).astype(bf16)
            if c == 1:
                w3T_s[0:896, :] = w3_v[:, 0:896].T
            if c == 2:
                w3T_s[896:F, :] = w3_v[:, 896:F].T
            if c == 3:
                w2T_s[...] = w2_v[...].T
                wo32 = wo_v[...].astype(f32)
                zrows = jnp.zeros((HP - DH, D), f32)
                parts = []
                for h in range(H):
                    parts.append(wo32[h * DH:(h + 1) * DH, :])
                    parts.append(zrows)
                woT_s[...] = jnp.concatenate(parts, axis=0).T.astype(bf16)

    q0 = pl.multiple_of(step * TQ, TQ)

    def qk_chunk(h, c, s_ref):
        s = _dot(k_s[h // 4, pl.ds(c * CK, CK), :], qp_s[h, :, pl.ds(q0, TQ)])
        s_ref[pl.ds(c * CK, CK), :] = s
        return jnp.max(s.reshape(CK // 8, 8, TQ), axis=0)

    def pv_chunk(h, c, s_ref, m):
        p = jnp.exp2(s_ref[pl.ds(c * CK, CK), :] - m).astype(bf16)
        return _dot(vt_s[h, :, pl.ds(c * CK, CK)], p)

    def attn_step(h, s_cur, m_cur, s_nxt, m_nxt):
        m = m_cur[...] if s_cur is not None else None
        mm = None
        acc = None
        for c in range(NC):
            if s_nxt is not None:
                mc = qk_chunk(h + 1, c, s_nxt)
                mm = mc if mm is None else jnp.maximum(mm, mc)
            if s_cur is not None:
                oc = pv_chunk(h, c, s_cur, m)
                acc = oc if acc is None else acc + oc
        if s_nxt is not None:
            m_nxt[...] = jnp.max(mm, axis=0, keepdims=True)
        if s_cur is not None:
            l = acc[DH:DH + 1, :]
            ot_s[h] = (acc * (1.0 / l)).astype(bf16)

    attn_step(-1, None, None, sa, ma)

    def body(t, carry):
        attn_step(2 * t, sa, ma, sb, mb)
        attn_step(2 * t + 1, sb, mb, sa, ma)
        return carry

    jax.lax.fori_loop(0, H // 2 - 1, body, 0)
    attn_step(H - 2, sa, ma, sb, mb)
    attn_step(H - 1, sb, mb, None, None)

    x = xt_s[:, pl.ds(q0, TQ)].astype(f32)
    parts = []
    for g, off in enumerate((-1, 1, -2, 2)):
        hw = ht_s[g * G:(g + 1) * G, pl.ds(q0, TQ + 2 * HALO)]
        parts.append(hw[:, HALO + off:HALO + off + TQ])
    hs = jnp.concatenate(parts, axis=0)
    x1 = x + _dot(w2T_s[...], hs)
    xn1 = _layernorm_t(x1).astype(bf16)
    h2 = _gelu(_dot(w3T_s[...], xn1)).astype(bf16)
    y = _dot(w4t_s[...], h2)
    a = _dot(woT_s[...], ot_s[...].reshape(H * HP, TQ))
    gate = g_s[:, pl.ds(q0, TQ)]
    out_ref[...] = (gate * a + (1.0 - gate) * (x1 + y)).astype(out_ref.dtype)


@jax.jit
def pallas_gated_mix__mha_block__mixer_s_mlp__prompt_kernel(
    A_x: jax.Array,
    A_wqkv: jax.Array,
    A_wo: jax.Array,
    B_x: jax.Array,
    B_w1: jax.Array,
    B_w2: jax.Array,
    B_w3: jax.Array,
    B_w4: jax.Array,
    gate_w: jax.Array,
):
    xt = A_x.reshape(T, D).T
    w4t = B_w4.T
    hbm = pl.BlockSpec(memory_space=pltpu.MemorySpace.HBM)

    out_t = pl.pallas_call(
        _kernel,
        grid=(T // TQ,),
        in_specs=[hbm] * 7 + [pl.BlockSpec((D,), lambda i: (0,))],
        out_specs=pl.BlockSpec((D, TQ), lambda i: (0, i)),
        out_shape=jax.ShapeDtypeStruct((D, T), bf16),
        scratch_shapes=[
            pltpu.VMEM((D, T), bf16),
            pltpu.VMEM((D, 3 * D), bf16),
            pltpu.VMEM((D, D), bf16),
            pltpu.VMEM((D, D), bf16),
            pltpu.VMEM((D, D), bf16),
            pltpu.VMEM((D, F), bf16),
            pltpu.VMEM((D, F), bf16),
            pltpu.SemaphoreType.DMA((8,)),
            pltpu.VMEM((3 * D + 16, D), bf16),
            pltpu.VMEM((D, D), bf16),
            pltpu.VMEM((D, D), bf16),
            pltpu.VMEM((F, D), bf16),
            pltpu.VMEM((D, H * HP), bf16),
            pltpu.VMEM((4, T, G), bf16),
            pltpu.VMEM((H, G, T), bf16),
            pltpu.VMEM((H, HP, T), bf16),
            pltpu.VMEM((D, T + 2 * HALO), bf16),
            pltpu.VMEM((1, T), f32),
            pltpu.VMEM((D + 8, TP), f32),
            pltpu.VMEM((T, TQ), f32),
            pltpu.VMEM((T, TQ), f32),
            pltpu.VMEM((1, TQ), f32),
            pltpu.VMEM((1, TQ), f32),
            pltpu.VMEM((H, HP, TQ), bf16),
        ],
        compiler_params=pltpu.CompilerParams(
            dimension_semantics=("arbitrary",),
            vmem_limit_bytes=100 * 1024 * 1024,
        ),
        name="gated_mix",
    )(xt, A_wqkv, A_wo, B_w1, B_w2, B_w3, w4t, gate_w)
    return out_t.T.reshape(1, T, D)
```

```python
import functools
import math

import jax
import jax.numpy as jnp
import jax.experimental.pallas as pl
import jax.experimental.pallas.tpu as pltpu

T = 2048
D = 448
H = 16
DH = 28
F = 1792
G = 112
HP = 32
TQ = 256
CK = 128
TP = 512
SL = 64
HT = 128
HALO = 128
EPS = 1e-5
QSCALE = (DH ** -0.5) * math.log2(math.e)
XA = 512
XB = 1536
XFIRST = 1
NLN0 = 4
ISSUE = (2, 3, 6, 10)
LAG = 3
TIE = 3
FC = 256
KC = 256
HV = 2
B1_AT = 4
B1_D = 2
W3_AT = 16
W3_STRIDE = 0
W4_STRIDE = 4
GROW = 3 * D

f32 = jnp.float32
bf16 = jnp.bfloat16
u32 = jnp.uint32


def _gelu(x):
    c = math.sqrt(2.0 / math.pi)
    inner = x * (c + (c * 0.044715) * (x * x))
    hx = 0.5 * x
    return hx + hx * jnp.tanh(inner)


def _layernorm_t(x):
    m = jnp.sum(x, axis=0, keepdims=True) * (1.0 / D)
    xc = x - m
    v = jnp.sum(xc * xc, axis=0, keepdims=True) * (1.0 / D)
    r = jax.lax.rsqrt(v + EPS)
    return x * r - m * r


def _dot(a, b):
    return jnp.dot(a, b, preferred_element_type=f32)


def _pack(x):
    return pltpu.bitcast(x, jnp.uint32)


def _unpack(x):
    return pltpu.bitcast(x, bf16)


def _kernel(xt_hbm, wqkv_hbm, wo_hbm, w1_hbm, w2_hbm, w3_hbm, w4t_hbm, gw_hbm,
            out_ref,
            xt_s, wqkv_v, wo_v, w1_v, w2_v, w3_v, w4t_s, gw_v, sems,
            wqkvT_s, w1T_s, w2T_s, w3T_s, woT_s,
            k_s, qp_s, vt_s, ht_s, g_s, tmp_s,
            sa, sb, ot_s, y_s, xn_s, h2_s, xn1_s):
    step = pl.program_id(0)
    NC = T // CK

    @pl.when(step == 0)
    def _prologue():
        cp_w1 = pltpu.make_async_copy(w1_hbm, w1_v, sems.at[0])
        cp_xa = pltpu.make_async_copy(xt_hbm.at[:, 0:XA], xt_s.at[:, 0:XA], sems.at[1])
        cp_xb = pltpu.make_async_copy(xt_hbm.at[:, XA:XB], xt_s.at[:, XA:XB], sems.at[2])
        cp_xc = pltpu.make_async_copy(xt_hbm.at[:, XB:], xt_s.at[:, XB:], sems.at[3])
        cp_wqkv = pltpu.make_async_copy(wqkv_hbm, wqkv_v, sems.at[4])
        cp_gw = pltpu.make_async_copy(gw_hbm, gw_v, sems.at[5])
        cp_w3 = pltpu.make_async_copy(w3_hbm, w3_v, sems.at[6])
        cp_w2 = pltpu.make_async_copy(w2_hbm, w2_v, sems.at[7])
        cp_wo = pltpu.make_async_copy(wo_hbm, wo_v, sems.at[8])
        cp_w4 = pltpu.make_async_copy(w4t_hbm, w4t_s, sems.at[9])
        order = ([cp_xa, cp_w1] if XFIRST else [cp_w1, cp_xa]) + [cp_xb, cp_xc, cp_wqkv, cp_gw, cp_w3, cp_w2, cp_wo, cp_w4]
        for cp in order[:ISSUE[0]]:
            cp.start()
        ht_s[:, 0:HALO] = jnp.zeros((D, HALO), bf16)
        ht_s[:, HALO + T:] = jnp.zeros((D, HALO), bf16)

        row_s = jax.lax.broadcasted_iota(jnp.int32, (SL, TP), 0)
        row_h = jax.lax.broadcasted_iota(jnp.int32, (HP, TP), 0)

        def ln_tile(j):
            xc = xt_s[:, j * HT:(j + 1) * HT]
            xn1_s[:, j * HT:(j + 1) * HT] = _pack(_layernorm_t(xc.astype(f32)).astype(bf16))

        def h_tile(j):
            xn = _unpack(xn1_s[:, j * HT:(j + 1) * HT])
            ht_s[:, HALO + j * HT:HALO + (j + 1) * HT] = _gelu(_dot(w1T_s[...], xn)).astype(bf16)

        def qkv_chunk(c):
            t0 = c * TP
            xc = xt_s[:, t0:t0 + TP]
            r = _dot(wqkvT_s[...], xc)
            for v in range(H // HV):
                g, odd = divmod(v, 2)
                lo = (G - SL) * odd
                qg = r[g * G + lo:g * G + lo + SL, :] * QSCALE
                for j in range(HV):
                    h0 = (odd * HV + j) * DH - lo
                    qm = jnp.where((row_s >= h0) & (row_s < h0 + DH), qg, 0.0)
                    for b in range(TP // TQ):
                        qp_s[t0 // TQ + b, v, :, j * TQ:(j + 1) * TQ] = _pack(
                            qm[:, b * TQ:(b + 1) * TQ].astype(bf16))
            for g in range(4):
                k_s[g, t0 // 2:(t0 + TP) // 2, :] = _pack(
                    r[D + g * G:D + (g + 1) * G, :].astype(bf16).T)
            tmp_s[...] = r[2 * D:3 * D + 8, :]
            for h in range(H):
                vh = tmp_s[h * DH:h * DH + HP, :]
                vh = jnp.where(row_h < DH, vh, jnp.where(row_h == DH, 1.0, 0.0))
                vt_s[h, :, t0:t0 + TP] = _pack(vh.astype(bf16))
            g_s[:, t0:t0 + TP] = jax.nn.sigmoid(r[GROW:GROW + 1, :])

        na, nb, nt = XA // HT, XB // HT, T // HT
        cp_xa.wait()
        for cp in order[ISSUE[0]:ISSUE[1]]:
            cp.start()
        for j in range(NLN0):
            ln_tile(j)
        cp_w1.wait()
        for cp in order[ISSUE[1]:ISSUE[2]]:
            cp.start()
        w1T_s[...] = w1_v[...].T
        for j in range(NLN0, na):
            ln_tile(j)
        for j in range(na - 1):
            h_tile(j)
        cp_xb.wait()
        for cp in order[ISSUE[2]:ISSUE[3]]:
            cp.start()
        for j in range(na, nb):
            ln_tile(j)
        for j in range(na - 1, nb - 1):
            h_tile(j)
        cp_xc.wait()
        cp_wqkv.wait()
        cp_gw.wait()
        for cp in order[ISSUE[3]:]:
            cp.start()
        row16 = jax.lax.broadcasted_iota(jnp.int32, (16, D), 0)
        gw = jnp.broadcast_to(gw_v[...].astype(f32).reshape(1, D), (16, D))
        wqkvT_s[GROW:GROW + 16, :] = jnp.where(row16 == 0, gw, 0.0).astype(bf16)
        wqkvT_s[0:GROW, :] = wqkv_v[...].T
        for j in range(nb, nt):
            ln_tile(j)
        for j in range(nb - 1, nt):
            h_tile(j)
        qkv_chunk(0)
        qkv_chunk(1)
        cp_w3.wait()
        cp_w2.wait()
        cp_wo.wait()
        cp_w4.wait()
        qkv_chunk(2)
        w3T_s[...] = w3_v[...].T
        qkv_chunk(3)
        w2T_s[...] = w2_v[...].T
        wo32 = wo_v[...].astype(f32)
        zrows = jnp.zeros((HP - DH, D), f32)
        parts = []
        for h in range(H):
            parts.append(wo32[h * DH:(h + 1) * DH, :])
            parts.append(zrows)
        woT_s[...] = jnp.concatenate(parts, axis=0).T.astype(bf16)

    q0 = pl.multiple_of(step * TQ, TQ)
    bufs = (sa, sb)
    NV = H // HV
    W = HV * TQ

    def qk_chunk(v, c):
        g, odd = divmod(v, 2)
        rhs = _unpack(qp_s[step, v])
        rows = slice(c * CK // 2, (c + 1) * CK // 2)
        if odd:
            rhs = jnp.concatenate([jnp.zeros((G - SL, W), bf16), rhs], axis=0)
            lhs = _unpack(k_s[g, rows, :])
        else:
            lhs = _unpack(k_s[g, rows, 0:SL])
        s = _dot(lhs, rhs)
        bufs[v % 2][c * CK:(c + 1) * CK, :] = s
        return jnp.max(s.reshape(CK // 8, 8, W), axis=0)

    def pv_chunk(v, c, m):
        outs = []
        for j in range(HV):
            mj = m[:, j * TQ:(j + 1) * TQ]
            mb = jnp.broadcast_to(mj[None], (CK // 8, 8, TQ)).reshape(CK, TQ)
            sj = bufs[v % 2][c * CK:(c + 1) * CK, j * TQ:(j + 1) * TQ]
            p = jnp.exp2(sj - mb).astype(bf16)
            outs.append(_dot(_unpack(vt_s[v * HV + j, :, c * CK:(c + 1) * CK]), p))
        return outs

    st = {}

    def b_part1():
        x = xt_s[:, pl.ds(q0, TQ)].astype(f32)
        parts = []
        for g, off in enumerate((-1, 1, -2, 2)):
            hw = ht_s[g * G:(g + 1) * G, pl.ds(q0, TQ + 2 * HALO)]
            parts.append(hw[:, HALO + off:HALO + off + TQ])
        hs = jnp.concatenate(parts, axis=0)
        x1 = x + _dot(w2T_s[...], hs)
        y_s[...] = x1
        st['mean'] = jnp.sum(x1, axis=0, keepdims=True) * (1.0 / D)

    def b_part1b():
        xc = y_s[...] - st['mean']
        var = jnp.sum(xc * xc, axis=0, keepdims=True) * (1.0 / D)
        st['rstd'] = jax.lax.rsqrt(var + EPS)

    def b_part1c():
        xn_s[...] = (y_s[...] * st['rstd'] - st['mean'] * st['rstd']).astype(bf16)

    def b_w3(i):
        h2_s[i * FC:(i + 1) * FC, :] = _gelu(
            _dot(w3T_s[i * FC:(i + 1) * FC, :], xn_s[...])).astype(bf16)

    def b_w4(i):
        y_s[...] += _dot(w4t_s[:, i * KC:(i + 1) * KC], h2_s[i * KC:(i + 1) * KC, :])

    total = NV * NC
    extra = {}
    extra.setdefault(B1_AT, []).append(b_part1)
    extra.setdefault(B1_AT + B1_D, []).append(b_part1b)
    extra.setdefault(B1_AT + 2 * B1_D, []).append(b_part1c)
    for i in range(F // FC):
        extra.setdefault(W3_AT + i * W3_STRIDE, []).append(functools.partial(b_w3, i))
    nw4 = F // KC
    for i in range(nw4):
        extra.setdefault(total + min(i * W4_STRIDE, NC + LAG), []).append(functools.partial(b_w4, i))

    mrun, mfin, acc, hist = {}, {}, {}, []
    for t in range(total + NC + LAG + 1):
        for fn in extra.get(t, ()):
            fn()
        if t < total:
            v, c = divmod(t, NC)
            mc = qk_chunk(v, c)
            mrun[v] = mc if c == 0 else jnp.maximum(mrun[v], mc)
            hist.append(mrun[v])
            if c == NC - 1:
                mfin[v] = jnp.broadcast_to(
                    jnp.max(mrun[v], axis=0, keepdims=True), (8, W))
        u = t - NC - LAG
        if 0 <= u < total:
            v, c = divmod(u, NC)
            m = mfin[v]
            if TIE and t - TIE < total:
                m = jnp.maximum(m, jnp.minimum(m, hist[t - TIE]))
            oc = pv_chunk(v, c, m)
            acc[v] = oc if c == 0 else [a_ + o_ for a_, o_ in zip(acc[v], oc)]
            if c == NC - 1:
                for j in range(HV):
                    l = acc[v][j][DH:DH + 1, :]
                    ot_s[v * HV + j] = (acc[v][j] * (1.0 / l)).astype(bf16)

    a = _dot(woT_s[...], ot_s[...].reshape(H * HP, TQ))
    gate = g_s[:, pl.ds(q0, TQ)]
    out_ref[...] = (gate * a + (1.0 - gate) * y_s[...]).astype(out_ref.dtype)


@jax.jit
def pallas_gated_mix__mha_block__mixer_s_mlp__prompt_kernel(
    A_x: jax.Array,
    A_wqkv: jax.Array,
    A_wo: jax.Array,
    B_x: jax.Array,
    B_w1: jax.Array,
    B_w2: jax.Array,
    B_w3: jax.Array,
    B_w4: jax.Array,
    gate_w: jax.Array,
):
    xt = A_x.reshape(T, D).T
    w4t = B_w4.T
    hbm = pl.BlockSpec(memory_space=pltpu.MemorySpace.HBM)

    out_t = pl.pallas_call(
        _kernel,
        grid=(T // TQ,),
        in_specs=[hbm] * 8,
        out_specs=pl.BlockSpec((D, TQ), lambda i: (0, i)),
        out_shape=jax.ShapeDtypeStruct((D, T), bf16),
        scratch_shapes=[
            pltpu.VMEM((D, T), bf16),
            pltpu.VMEM((D, 3 * D), bf16),
            pltpu.VMEM((D, D), bf16),
            pltpu.VMEM((D, D), bf16),
            pltpu.VMEM((D, D), bf16),
            pltpu.VMEM((D, F), bf16),
            pltpu.VMEM((D, F), bf16),
            pltpu.VMEM((D,), bf16),
            pltpu.SemaphoreType.DMA((10,)),
            pltpu.VMEM((3 * D + 16, D), bf16),
            pltpu.VMEM((D, D), bf16),
            pltpu.VMEM((D, D), bf16),
            pltpu.VMEM((F, D), bf16),
            pltpu.VMEM((D, H * HP), bf16),
            pltpu.VMEM((4, T // 2, G), u32),
            pltpu.VMEM((T // TQ, H // HV, SL // 2, HV * TQ), u32),
            pltpu.VMEM((H, HP // 2, T), u32),
            pltpu.VMEM((D, T + 2 * HALO), bf16),
            pltpu.VMEM((1, T), f32),
            pltpu.VMEM((D + 8, TP), f32),
            pltpu.VMEM((T, HV * TQ), f32),
            pltpu.VMEM((T, HV * TQ), f32),
            pltpu.VMEM((H, HP, TQ), bf16),
            pltpu.VMEM((D, TQ), f32),
            pltpu.VMEM((D, TQ), bf16),
            pltpu.VMEM((F, TQ), bf16),
            pltpu.VMEM((D // 2, T), u32),
        ],
        compiler_params=pltpu.CompilerParams(
            dimension_semantics=("arbitrary",),
            vmem_limit_bytes=100 * 1024 * 1024,
        ),
        name="gated_mix",
    )(xt, A_wqkv, A_wo, B_w1, B_w2, B_w3, w4t, gate_w)
    return out_t.T.reshape(1, T, D)
```

```python
import functools
import math

import jax
import jax.numpy as jnp
import jax.experimental.pallas as pl
import jax.experimental.pallas.tpu as pltpu

T = 2048
D = 448
H = 16
DH = 28
F = 1792
G = 112
HP = 32
TQ = 256
CK = 128
TP = 512
SL = 64
HT = 128
HALO = 128
HV = 2
EPS = 1e-5
QSCALE = (DH ** -0.5) * math.log2(math.e)
GROW = 3 * D

VRS = (48, 48, 48, 48)
HLATE = 0
KB0 = 24
KFIRST = 1
QCC = (2, 3)
X0 = 0
X1 = 128
XPAUSE = (98, 99)
GR = 8
ORD0 = 2
QEVERY = 8
XP = 4
LAG = 2
KC = 256
B1_AT = 0
W3_AT = (100, 100)
W4_AT = 102
W4_STRIDE = 0
WTA = 10
WT3 = 6
WT2 = 10
WTE = 10
XG = 4
XT = 1
WT4 = 10
X0T = 384
W1A = 256
XA = 768
XB = 1536
L_HI = 2.0 ** 110
L_LO = 2.0 ** -60

NOFF = sum(VRS)
NVT = len(VRS)
VOFF = [sum(VRS[:i]) for i in range(NVT + 1)]
NC = T // CK
NV = H // HV
W = HV * TQ
NT = TQ // 128
NSTEP = T // TQ
HK = H * HP // 2

f32 = jnp.float32
bf16 = jnp.bfloat16
u32 = jnp.uint32
i32 = jnp.int32


def _gelu(x):
    c = math.sqrt(2.0 / math.pi)
    inner = x * (c + (c * 0.044715) * (x * x))
    hx = 0.5 * x
    return hx + hx * jnp.tanh(inner)


def _layernorm_t(x):
    m = jnp.sum(x, axis=0, keepdims=True) * (1.0 / D)
    xc = x - m
    v = jnp.sum(xc * xc, axis=0, keepdims=True) * (1.0 / D)
    r = jax.lax.rsqrt(v + EPS)
    return x * r - m * r


def _dot(a, b):
    return jnp.dot(a, b, preferred_element_type=f32)


def _pack(x):
    return pltpu.bitcast(x, u32)


def _unpack(x):
    return pltpu.bitcast(x, bf16)


def _after(x, dep):
    return jnp.maximum(x, jnp.minimum(x, dep))


def _kernel(xt_hbm, wqkv_hbm, wo_hbm, w1_hbm, w2_hbm, w3_hbm, w4t_hbm, gw_hbm,
            out_ref,
            xt_s, wqkv_v, wo_v, w1_v, w2_v, w3_v, w4t_s, gw_v, sems,
            wqkvT_s, w1T_s, w2T_s, w3T_s, woT_s,
            k_s, qp_s, vt_s, ht_s, g_s, tmp_s,
            ot_s, y_s, xn_s, h2_s, xn1_s, qf_s, kb_s, sv_s, qc_s, qs_s,
            fs_s, fr_s, hs_s, mx_s):
    step = pl.program_id(0)

    def fill_qc(blk, r8, tl, dep):
        x8 = _after(qf_s[blk * NT + tl, r8 * 8:(r8 + 1) * 8, :], dep)
        qc_s[tl, r8 * 8:(r8 + 1) * 8] = jnp.stack(
            [jnp.broadcast_to(x8[i:i + 1, :], (8, 128)) for i in range(8)])

    def fill_qs(blk, v, part, dep):
        x = pltpu.bitcast(qp_s[blk, v, part * 8:(part + 1) * 8, :], i32)
        di = jnp.concatenate([pltpu.bitcast(dep, i32)] * (W // 128), axis=1)
        qs_s[v, part * 8:(part + 1) * 8, :] = pltpu.bitcast(_after(x, di), u32)

    def fill_hs(blk, r8, dep):
        off = (-1, 1, -2, 2)[r8 // 7]
        lo = 0 if off < 0 else HALO
        t0 = blk * NT + lo // HALO
        hw = jnp.concatenate(
            [ht_s[t0 + i, r8 * 8:(r8 + 1) * 8, :] for i in range(NT + 1)], axis=1)
        hw = pltpu.bitcast(hw, i32)
        if dep is not None:
            di = jnp.concatenate([pltpu.bitcast(dep, i32)] * (NT + 1), axis=1)
            hw = _after(hw, di)
        hs_s[r8 * 8:(r8 + 1) * 8, :] = pltpu.bitcast(
            hw[:, HALO + off - lo:HALO + off - lo + TQ], u32)

    def qk_rhs(v, slab, last):
        zeros = jnp.zeros((G - SL, W), bf16)
        parts = [zeros, slab] if v % 2 else [slab, zeros]
        return jnp.concatenate(parts + [last], axis=0)

    @pl.when(step == 0)
    def _prologue():
        cp_x0 = pltpu.make_async_copy(xt_hbm.at[:, 0:X0T], xt_s.at[:, 0:X0T], sems.at[0])
        cp_w1a = pltpu.make_async_copy(w1_hbm.at[:, 0:W1A], w1_v.at[:, 0:W1A], sems.at[1])
        cp_w1b = pltpu.make_async_copy(w1_hbm.at[:, W1A:], w1_v.at[:, W1A:], sems.at[10])
        cp_xa = pltpu.make_async_copy(xt_hbm.at[:, X0T:XA], xt_s.at[:, X0T:XA], sems.at[11])
        cp_xb = pltpu.make_async_copy(xt_hbm.at[:, XA:XB], xt_s.at[:, XA:XB], sems.at[2])
        cp_xc = pltpu.make_async_copy(xt_hbm.at[:, XB:], xt_s.at[:, XB:], sems.at[3])
        cp_wqkv = pltpu.make_async_copy(wqkv_hbm, wqkv_v, sems.at[4])
        cp_gw = pltpu.make_async_copy(gw_hbm, gw_v, sems.at[5])
        cp_w3 = pltpu.make_async_copy(w3_hbm, w3_v, sems.at[6])
        cp_w2 = pltpu.make_async_copy(w2_hbm, w2_v, sems.at[7])
        cp_wo = pltpu.make_async_copy(wo_hbm, wo_v, sems.at[8])
        cp_w4 = pltpu.make_async_copy(w4t_hbm, w4t_s, sems.at[9])
        cp_x0.start()
        cp_w1a.start()
        cp_w1b.start()
        cp_xa.start()
        ht_s[0, 0:D // 2, :] = jnp.zeros((D // 2, HALO), u32)
        ht_s[T // HT + 1, 0:D // 2, :] = jnp.zeros((D // 2, HALO), u32)

        row_s = jax.lax.broadcasted_iota(i32, (SL, TP), 0)
        row_h = jax.lax.broadcasted_iota(i32, (HP, TP), 0)
        ones_row = jnp.where(jax.lax.broadcasted_iota(i32, (16, TP), 0) == 0, 1.0, 0.0)

        def ln_tile(j):
            xc = xt_s[:, j * HT:(j + 1) * HT]
            xn1_s[:, j * HT:(j + 1) * HT] = _pack(_layernorm_t(xc.astype(f32)).astype(bf16))

        def h_tile(j, r0=0, r1=D):
            xn = _unpack(xn1_s[:, j * HT:(j + 1) * HT])
            ht_s[j + 1, r0 // 2:r1 // 2, :] = _pack(
                _gelu(_dot(_unpack(w1T_s[r0 // 2:r1 // 2]), xn)).astype(bf16))

        def vpu_keys(g):
            return jnp.concatenate(
                [k_s[g, tl * CK // 2:(tl * CK + VRS[tl]) // 2, :] for tl in range(NVT)], axis=0)

        def kb_pieces(p_lo, p_hi):
            for p in range(p_lo, p_hi):
                g, d0 = divmod(p * 8, G)
                kp = vpu_keys(g)
                cols = jnp.concatenate(
                    [jnp.broadcast_to(kp[:, d:d + 1], (NOFF // 2, 128))
                     for d in range(d0, d0 + 8)], axis=0)
                kb_s[p * 8:(p + 1) * 8] = _unpack(cols).astype(f32).reshape(8, NOFF, 128)

        def k_part(c, rk):
            t0 = c * TP
            for g in range(4):
                kt = jnp.concatenate([rk[g * G:(g + 1) * G, :], ones_row], axis=0)
                k_s[g, t0 // 2:(t0 + TP) // 2, :] = _pack(kt.astype(bf16).T)

        def qkv_chunk(c, with_k=True):
            t0 = c * TP
            xc = xt_s[:, t0:t0 + TP]
            if with_k:
                r = _dot(_unpack(wqkvT_s[...]), xc)
                k_part(c, r[D:2 * D])
                rv = r[2 * D:]
            else:
                lhs = jnp.concatenate([wqkvT_s[0:D // 2], wqkvT_s[D:]], axis=0)
                r = _dot(_unpack(lhs), xc)
                rv = r[D:]
            qf = r[0:D, :] * QSCALE
            for v in range(NV):
                g, odd = divmod(v, 2)
                lo = (G - SL) * odd
                qg = qf[g * G + lo:g * G + lo + SL, :]
                for j in range(HV):
                    h0 = (odd * HV + j) * DH - lo
                    qm = jnp.where((row_s >= h0) & (row_s < h0 + DH), qg, 0.0)
                    for b in range(TP // TQ):
                        qp_s[t0 // TQ + b, v, :, j * TQ:(j + 1) * TQ] = _pack(
                            qm[:, b * TQ:(b + 1) * TQ].astype(bf16))
            for tl in range(TP // 128):
                if t0 // 128 + tl >= NT:
                    qf_s[t0 // 128 + tl, 0:D, :] = qf[:, tl * 128:(tl + 1) * 128]
            tmp_s[...] = rv[0:D + 8, :]
            for h in range(H):
                vh = tmp_s[h * DH:h * DH + HP, :]
                vh = jnp.where(row_h < DH, vh, jnp.where(row_h == DH, 1.0, 0.0))
                vt_s[h, :, t0:t0 + TP] = _pack(vh.astype(bf16))
            g_s[:, t0:t0 + TP] = jax.nn.sigmoid(rv[D:D + 1, :])
            if c in QCC:
                for i in range(56):
                    r8, tl = QCC.index(c) * 28 + i // 2, i % 2
                    rr = (i % 14) * 96
                    dep = r[rr:rr + 8, (i // 14) * 128:(i // 14 + 1) * 128]
                    fill_qc(1, r8, tl, dep)

        na, nb, nt = XA // HT, XB // HT, T // HT
        n0 = X0T // HT
        cp_x0.wait()
        for j in range(n0):
            ln_tile(j)
        cp_w1a.wait()
        cp_xb.start()
        w1T_s[0:W1A // 2] = _pack(w1_v[:, 0:W1A].T)
        for j in range(n0 - 1):
            h_tile(j, 0, W1A)
        cp_w1b.wait()
        cp_xa.wait()
        cp_xc.start()
        cp_wqkv.start()
        cp_gw.start()
        h_tile(n0 - 1, 0, W1A)
        w1T_s[W1A // 2:] = _pack(w1_v[:, W1A:].T)
        for j in range(n0, na):
            ln_tile(j)
        for j in range(n0):
            h_tile(j, W1A, D)
        for j in range(n0, na - 1):
            h_tile(j)
        cp_xb.wait()
        cp_w3.start()
        cp_w2.start()
        cp_wo.start()
        cp_w4.start()
        for j in range(na, nb):
            ln_tile(j)
        for j in range(na - 1, nb - 1):
            h_tile(j)
        cp_xc.wait()
        cp_wqkv.wait()
        cp_gw.wait()
        row16 = jax.lax.broadcasted_iota(i32, (16, D), 0)
        gw = jnp.broadcast_to(gw_v[...].astype(f32).reshape(1, D), (16, D))
        wqkvT_s[GROW // 2:GROW // 2 + 8, :] = _pack(jnp.where(row16 == 0, gw, 0.0).astype(bf16))
        wqkvT_s[0:GROW // 2, :] = _pack(wqkv_v[...].T)
        for j in range(nb, nt):
            ln_tile(j)
        for j in range(nb - 1, nt - HLATE):
            h_tile(j)
        if KFIRST:
            k_part(0, _dot(_unpack(wqkvT_s[D // 2:D]), xt_s[:, 0:TP]))
            kb_pieces(0, KB0)
            for j in range(nt - HLATE, nt):
                h_tile(j)
            qkv_chunk(0, with_k=False)
        else:
            qkv_chunk(0)
            kb_pieces(0, KB0)
            for j in range(nt - HLATE, nt):
                h_tile(j)
        qkv_chunk(1)
        cp_w3.wait()
        cp_w2.wait()
        cp_wo.wait()
        cp_w4.wait()
        kb_pieces(KB0, D // 8)
        qkv_chunk(2)
        w3T_s[...] = _pack(w3_v[...].T)
        qkv_chunk(3)
        zlast = jnp.zeros((16, W), bf16)
        for v in range(NV):
            sv0 = _dot(_unpack(vpu_keys(v // 2)), qk_rhs(v, _unpack(qp_s[0, v]), zlast))
            sv_s[v] = sv0
            mx_s[v] = jnp.max(sv0.reshape(NOFF // 8, 8, W), axis=0)
        qs_s[...] = qp_s[0]
        for r8 in range(D // 16):
            fill_hs(0, r8, None)
        w2T_s[...] = _pack(w2_v[...].T)
        wo32 = wo_v[...].astype(f32)
        zrows = jnp.zeros((HP - DH, D), f32)
        parts = []
        for h in range(H):
            parts.append(wo32[h * DH:(h + 1) * DH, :])
            parts.append(zrows)
        woT_s[...] = _pack(jnp.concatenate(parts, axis=0).T.astype(bf16))

    q0 = pl.multiple_of(step * TQ, TQ)
    gate = g_s[:, pl.ds(q0, TQ)]
    st = {}

    XK = XG * 8

    def x_block(v, j, tl, b, deps):
        h = v * HV + j
        feat = slice(h * DH, (h + 1) * DH)
        qa = qc_s[tl:tl + XT, feat]
        ng = DH // XP
        q = qa.reshape(XT, ng, XP, 8, 128)
        q0_ = _after(q[:, :, 0:1], jnp.stack(deps)[None, :, None])
        q = jnp.concatenate([q0_, q[:, :, 1:]], axis=2).reshape(XT, DH, 1, 8, 128)
        kb = kb_s[feat, b * XK:(b + 1) * XK, :].reshape(1, DH, XG, 8, 128)
        sx = jnp.sum(kb * q, axis=1)
        mx = jnp.max(sx, axis=1)
        st['xmx'] = mx if b == 0 else jnp.maximum(st['xmx'], mx)
        for i in range(XT):
            c0 = j * TQ + (tl + i) * 128
            sv_s[v, b * XK:(b + 1) * XK, c0:c0 + 128] = sx[i].reshape(XK, 128)
            if b == NOFF // XK - 1:
                mx_s[v, :, c0:c0 + 128] = st['xmx'][i]

    xlist = [(v, j, tl, b) for v in range(NV) for j in range(HV) for tl in range(0, NT, XT)
             for b in range(NOFF // XK)]
    npieces = len(xlist) * (DH // XP)
    xstate = dict(done=0, gate=0, started=-1, n=0)
    xdeps = []
    nxt1 = jnp.minimum(step + 1, NSTEP - 1)
    nxt2 = jnp.minimum(step + 2, NSTEP - 1)
    qtasks = [functools.partial(fill_qc, nxt1, r8, tl)
              for r8 in range((NV - 1) * 7, NV * 7) for tl in range(NT)]

    def side_work(res, weight):
        for r_ in range(0, res.shape[0], GR):
            dep = res[r_:r_ + 8, 0:128]
            xstate['gate'] += weight
            if (xlist and weight and xlist[0][0] <= xstate['started']
                    and xstate['done'] * NGATE < npieces * xstate['gate']):
                xstate['done'] += 1
                xdeps.append(dep)
                if len(xdeps) == DH // XP:
                    xb = xlist.pop(0)
                    x_block(*xb, list(xdeps))
                    xdeps.clear()
                    if xlist and xlist[0][0] != xb[0]:
                        qtasks.extend(functools.partial(fill_qc, nxt2, r8, tl)
                                      for r8 in range(xb[0] * 7, (xb[0] + 1) * 7)
                                      for tl in range(NT))
            xstate['n'] += 1
            if qtasks and xstate['n'] % QEVERY == 0:
                qtasks.pop(0)(dep)

    def b_part1():
        x = xt_s[:, pl.ds(q0, TQ)].astype(f32)
        zs = [_dot(_unpack(w2T_s[...]), _unpack(hs_s[:, tl * 128:(tl + 1) * 128]))
              for tl in range(NT)]
        for z in zs:
            side_work(z, WT2)
        x1 = x + jnp.concatenate(zs, axis=1)
        y_s[...] = x1
        xn_s[...] = _pack(_layernorm_t(x1).astype(bf16))
        qtasks.extend(functools.partial(fill_hs, nxt1, r8) for r8 in range(D // 16))

    def b_w3(tl):
        z = _dot(_unpack(w3T_s[...]), _unpack(xn_s[:, tl * 128:(tl + 1) * 128]))
        h2_s[:, tl * 128:(tl + 1) * 128] = _pack(_gelu(z).astype(bf16))
        side_work(z, WT3)

    def b_w4(i, wt):
        yi = y_s[...] + _dot(w4t_s[:, i * KC:(i + 1) * KC],
                             _unpack(h2_s[i * KC // 2:(i + 1) * KC // 2, :]))
        y_s[...] = yi
        side_work(yi, wt)

    def b_wo_a():
        a_ = _dot(_unpack(woT_s[:, 0:HK]), _unpack(ot_s[0:H // 2].reshape(HK // 2, TQ)))
        st['a'] = gate * a_
        side_work(a_, WTE)

    total = NV * NC
    nw4 = F // KC
    extra = {}
    extra.setdefault(B1_AT, []).append(b_part1)
    for tl in range(NT):
        extra.setdefault(W3_AT[tl], []).append(functools.partial(b_w3, tl))
    for i in range(nw4 - 1):
        extra.setdefault(W4_AT + i * W4_STRIDE, []).append(functools.partial(b_w4, i, WT4))
    extra.setdefault(total, []).append(b_wo_a)
    extra.setdefault(total + LAG, []).append(functools.partial(b_w4, nw4 - 1, WTE))

    order = list(range(NVT, NC))
    for i in range(NVT):
        order.insert(ORD0 + i * (NC // NVT), i)
    nrows = [CK - (VRS[kt] if kt < NVT else 0) for kt in order]
    wslot = [0 if (t < X0 or t >= X1 or t in XPAUSE) else WTA for t in range(total)]
    NGATE = (sum(wslot[t] * (nrows[t % NC] // GR) for t in range(total))
             + NT * WT3 * (F // GR) + ((nw4 - 1) * WT4 + NT * WT2 + 2 * WTE) * (D // GR))
    row16w = jax.lax.broadcasted_iota(i32, (16, W), 0)
    rhs, svm, ptile, acc = {}, {}, {}, {}
    lmax = lmin = None
    for t in range(total + LAG + 1):
        if t < total and t % NC == 0:
            v = t // NC
            sv = sv_s[v]
            m0 = jnp.max(mx_s[v], axis=0, keepdims=True)
            m0 = m0.astype(bf16).astype(f32)
            last = jnp.where(row16w == 0, -m0, 0.0).astype(bf16)
            rhs[v] = qk_rhs(v, _unpack(qs_s[v]), last)
            svm[v] = sv - m0
            xstate['started'] = v
        for fn in extra.get(t, ()):
            fn()
        if t < total:
            v, c = divmod(t, NC)
            kt = order[c]
            lo = kt * CK + (VRS[kt] if kt < NVT else 0)
            s = _dot(_unpack(k_s[v // 2, lo // 2:(kt + 1) * CK // 2, :]), rhs[v])
            ps = []
            for j in range(HV):
                cols = slice(j * TQ, (j + 1) * TQ)
                sj = s[:, cols]
                if kt < NVT:
                    sj = jnp.concatenate([svm[v][VOFF[kt]:VOFF[kt + 1], cols], sj], axis=0)
                ps.append(jnp.exp2(sj).astype(bf16))
            ptile[t] = ps
            if c == NC - 1:
                qtasks[0:0] = [functools.partial(fill_qs, nxt1, v, p_) for p_ in range(SL // 16)]
            side_work(s, wslot[t])
        u = t - LAG
        if 0 <= u < total:
            v, c = divmod(u, NC)
            kt = order[c]
            oc = [_dot(_unpack(vt_s[v * HV + j, :, kt * CK:(kt + 1) * CK]), ptile[u][j])
                  for j in range(HV)]
            acc[v] = oc if c == 0 else [a_ + o_ for a_, o_ in zip(acc[v], oc)]
            if c == NC - 1:
                for j in range(HV):
                    l = acc[v][j][DH:DH + 1, :]
                    am = jnp.max(jnp.abs(acc[v][j]).reshape(HP // 8, 8, TQ), axis=0)
                    lmax = am if lmax is None else jnp.maximum(lmax, am)
                    lmin = l if lmin is None else jnp.minimum(lmin, l)
                    ot_s[v * HV + j] = _pack((acc[v][j] * (1.0 / l)).astype(bf16))
    while qtasks:
        qtasks.pop(0)(oc[0][0:8, 0:128])
    assert not xlist

    rest = st['a'] + (1.0 - gate) * y_s[...]
    a = _dot(_unpack(woT_s[:, HK:]), _unpack(ot_s[H // 2:].reshape(HK // 2, TQ)))
    out_ref[...] = (gate * a + rest).astype(out_ref.dtype)

    safe = jnp.where((lmax < L_HI) & (lmin > L_LO), 1.0, 0.0)
    unsafe = jnp.min(safe) < 0.5

    @pl.when(unsafe)
    def _fallback():
        def head_pair(v, carry):
            fr_s[...] = jnp.zeros((CK // 2, W), u32)
            off = pl.multiple_of((v % 2) * ((G - SL) // 2), 8)
            fr_s[pl.ds(off, SL // 2), :] = qp_s[step, v]

            def scores(c, m):
                r0 = pl.multiple_of(c * CK, CK)
                s = _dot(_unpack(k_s[v // 2, pl.ds(pl.multiple_of(c * (CK // 2), CK // 2), CK // 2), :]),
                         _unpack(fr_s[...]))
                fs_s[pl.ds(r0, CK), :] = s
                return jnp.maximum(m, jnp.max(s, axis=0, keepdims=True))

            m = jax.lax.fori_loop(0, NC, scores, jnp.full((1, W), -jnp.inf, f32))

            def values(c, o):
                r0 = pl.multiple_of(c * CK, CK)
                p = jnp.exp2(fs_s[pl.ds(r0, CK), :] - m)
                return tuple(
                    o[j] + _dot(_unpack(vt_s[v * HV + j, :, pl.ds(r0, CK)]),
                                p[:, j * TQ:(j + 1) * TQ].astype(bf16))
                    for j in range(HV))

            o = jax.lax.fori_loop(0, NC, values,
                                  tuple(jnp.zeros((HP, TQ), f32) for _ in range(HV)))
            for j in range(HV):
                ot_s[v * HV + j] = _pack((o[j] * (1.0 / o[j][DH:DH + 1, :])).astype(bf16))
            return carry

        jax.lax.fori_loop(0, NV, head_pair, 0)
        a2 = _dot(_unpack(woT_s[...]), _unpack(ot_s[...].reshape(HK, TQ)))
        out_ref[...] = (gate * a2 + (1.0 - gate) * y_s[...]).astype(out_ref.dtype)


@jax.jit
def pallas_gated_mix__mha_block__mixer_s_mlp__prompt_kernel(
    A_x: jax.Array,
    A_wqkv: jax.Array,
    A_wo: jax.Array,
    B_x: jax.Array,
    B_w1: jax.Array,
    B_w2: jax.Array,
    B_w3: jax.Array,
    B_w4: jax.Array,
    gate_w: jax.Array,
):
    xt = A_x.reshape(T, D).T
    w4t = B_w4.T
    hbm = pl.BlockSpec(memory_space=pltpu.MemorySpace.HBM)

    out_t = pl.pallas_call(
        _kernel,
        grid=(NSTEP,),
        in_specs=[hbm] * 8,
        out_specs=pl.BlockSpec((D, TQ), lambda i: (0, i)),
        out_shape=jax.ShapeDtypeStruct((D, T), bf16),
        scratch_shapes=[
            pltpu.VMEM((D, T), bf16),
            pltpu.VMEM((D, 3 * D), bf16),
            pltpu.VMEM((D, D), bf16),
            pltpu.VMEM((D, D), bf16),
            pltpu.VMEM((D, D), bf16),
            pltpu.VMEM((D, F), bf16),
            pltpu.VMEM((D, F), bf16),
            pltpu.VMEM((D,), bf16),
            pltpu.SemaphoreType.DMA((12,)),
            pltpu.VMEM((GROW // 2 + 8, D), u32),
            pltpu.VMEM((D // 2, D), u32),
            pltpu.VMEM((D // 2, D), u32),
            pltpu.VMEM((F // 2, D), u32),
            pltpu.VMEM((D // 2, H * HP), u32),
            pltpu.VMEM((4, T // 2, 128), u32),
            pltpu.VMEM((NSTEP, NV, SL // 2, W), u32),
            pltpu.VMEM((H, HP // 2, T), u32),
            pltpu.VMEM((T // HT + 2, 256, HT), u32),
            pltpu.VMEM((1, T), f32),
            pltpu.VMEM((D + 8, TP), f32),
            pltpu.VMEM((H, HP // 2, TQ), u32),
            pltpu.VMEM((D, TQ), f32),
            pltpu.VMEM((D // 2, TQ), u32),
            pltpu.VMEM((F // 2, TQ), u32),
            pltpu.VMEM((D // 2, T), u32),
            pltpu.VMEM((T // 128, 512, 128), f32),
            pltpu.VMEM((D, NOFF, 128), f32),
            pltpu.VMEM((NV, NOFF, W), f32),
            pltpu.VMEM((NT, D, 8, 128), f32),
            pltpu.VMEM((NV, SL // 2, W), u32),
            pltpu.VMEM((T, W), f32),
            pltpu.VMEM((CK // 2, W), u32),
            pltpu.VMEM((D // 2, TQ), u32),
            pltpu.VMEM((NV, 8, W), f32),
        ],
        compiler_params=pltpu.CompilerParams(
            dimension_semantics=("arbitrary",),
            vmem_limit_bytes=120 * 1024 * 1024,
        ),
        name="gated_mix",
    )(xt, A_wqkv, A_wo, B_w1, B_w2, B_w3, w4t, gate_w)
    return out_t.T.reshape(1, T, D)
```

```python
import functools
import math

import jax
import jax.numpy as jnp
import jax.experimental.pallas as pl
import jax.experimental.pallas.tpu as pltpu

T = 2048
D = 448
H = 16
DH = 28
F = 1792
G = 112
HP = 32
TQ = 256
CK = 128
TP = 512
SL = 64
HT = 128
HV = 2
KC = 256
EPS = 1e-5
QSCALE = (DH ** -0.5) * math.log2(math.e)
GROW = 3 * D
L_HI = 2.0 ** 110
L_LO = 2.0 ** -60

NVT = 2
XK = 32
XP = 4
MB = 4

X0T = 256
W1A = 256
XA = 640
XB = 1536
HLATE = 3
KB0 = 15
QCC = (2, 3)
GR = 8
QEVERY = 8
FPOS = (2, 5)
WSL = (6, 4, 8, 10, 6, 8, 10, 10, 10, 10, 10, 10, 10, 10)
WT2 = 4
WT3 = 7
WT4 = 7
WTE = 7
W3_BACK = 2
NPAUSE = 2

NOFF = NVT * CK
NC = T // CK
NU = NC - NVT
NV = H // HV
W = HV * TQ
NT = TQ // 128
NSTEP = T // TQ
HK = H * HP // 2

f32 = jnp.float32
bf16 = jnp.bfloat16
u32 = jnp.uint32
i32 = jnp.int32


def _gelu(x):
    c = math.sqrt(2.0 / math.pi)
    inner = x * (c + (c * 0.044715) * (x * x))
    hx = 0.5 * x
    return hx + hx * jnp.tanh(inner)


def _layernorm_t(x):
    m = jnp.sum(x, axis=0, keepdims=True) * (1.0 / D)
    xc = x - m
    v = jnp.sum(xc * xc, axis=0, keepdims=True) * (1.0 / D)
    r = jax.lax.rsqrt(v + EPS)
    return x * r - m * r


def _dot(a, b):
    return jnp.dot(a, b, preferred_element_type=f32)


def _pack(x):
    return pltpu.bitcast(x, u32)


def _unpack(x):
    return pltpu.bitcast(x, bf16)


def _kernel(xt_hbm, wqkv_hbm, wo_hbm, w1_hbm, w2_hbm, w3_hbm, w4t_hbm, gw_hbm,
            out_ref,
            xt_s, wqkv_v, wo_v, w1_v, w2_v, w3_v, w4t_s, gw_v, sems,
            wqkvT_s, w1T_s, w2T_s, w3T_s, woT_s,
            k_s, qp_s, vt_s, ht_s, g_s,
            ot_s, y_s, xn_s, h2_s, xn1_s, qf_s, kb_s, sv_s, qc_s, qs_s,
            fs_s, fr_s, hs_s, mx_s):
    step = pl.program_id(0)
    true8 = jax.lax.broadcasted_iota(i32, (8, 128), 1) >= -step

    def _after(x, dep):
        reps = x.shape[-1] // 128
        m = true8 if reps == 1 else jnp.concatenate([true8] * reps, axis=1)
        return jnp.where(m, x, dep)

    def fill_qc(blk, r8, tl, dep):
        x8 = _after(qf_s[blk * NT + tl, r8 * 8:(r8 + 1) * 8, :], dep)
        qc_s[tl, r8 * 8:(r8 + 1) * 8] = jnp.stack(
            [jnp.broadcast_to(x8[i:i + 1, :], (8, 128)) for i in range(8)])

    def fill_qs(blk, v, part, dep):
        x = pltpu.bitcast(qp_s[blk, v, part * 8:(part + 1) * 8, :], i32)
        di = jnp.concatenate([pltpu.bitcast(dep, i32)] * (W // 128), axis=1)
        qs_s[v, part * 8:(part + 1) * 8, :] = pltpu.bitcast(_after(x, di), u32)

    def fill_hs(blk, r8, dep):
        off = (-1, 1, -2, 2)[r8 // 7]
        lo = 0 if off < 0 else 1
        hw = jnp.concatenate(
            [ht_s[blk * NT + lo + i, r8 * 8:(r8 + 1) * 8, :] for i in range(NT + 1)], axis=1)
        hw = pltpu.bitcast(hw, i32)
        if dep is not None:
            di = jnp.concatenate([pltpu.bitcast(dep, i32)] * (NT + 1), axis=1)
            hw = _after(hw, di)
        c0 = (1 - lo) * HT + off
        hs_s[r8 * 8:(r8 + 1) * 8, :] = pltpu.bitcast(hw[:, c0:c0 + TQ], u32)

    def qk_rhs(v, slab, last):
        zeros = jnp.zeros((G - SL, W), bf16)
        parts = [zeros, slab] if v % 2 else [slab, zeros]
        return jnp.concatenate(parts + [last], axis=0)

    @pl.when(step == 0)
    def _prologue():
        cp_x0 = pltpu.make_async_copy(xt_hbm.at[:, 0:X0T], xt_s.at[:, 0:X0T], sems.at[0])
        cp_w1a = pltpu.make_async_copy(w1_hbm.at[:, 0:W1A], w1_v.at[:, 0:W1A], sems.at[1])
        cp_w1b = pltpu.make_async_copy(w1_hbm.at[:, W1A:], w1_v.at[:, W1A:], sems.at[2])
        cp_xa = pltpu.make_async_copy(xt_hbm.at[:, X0T:XA], xt_s.at[:, X0T:XA], sems.at[3])
        cp_xb = pltpu.make_async_copy(xt_hbm.at[:, XA:XB], xt_s.at[:, XA:XB], sems.at[4])
        cp_xc = pltpu.make_async_copy(xt_hbm.at[:, XB:], xt_s.at[:, XB:], sems.at[5])
        cp_wqkv = pltpu.make_async_copy(wqkv_hbm, wqkv_v, sems.at[6])
        cp_gw = pltpu.make_async_copy(gw_hbm, gw_v, sems.at[7])
        cp_w3 = pltpu.make_async_copy(w3_hbm, w3_v, sems.at[8])
        cp_w2 = pltpu.make_async_copy(w2_hbm, w2_v, sems.at[9])
        cp_wo = pltpu.make_async_copy(wo_hbm, wo_v, sems.at[10])
        cp_w4 = pltpu.make_async_copy(w4t_hbm, w4t_s, sems.at[11])
        cp_x0.start()
        cp_w1a.start()
        cp_w1b.start()
        cp_xa.start()
        ht_s[0, 0:D // 2, :] = jnp.zeros((D // 2, HT), u32)
        ht_s[T // HT + 1, 0:D // 2, :] = jnp.zeros((D // 2, HT), u32)

        row_s = jax.lax.broadcasted_iota(i32, (SL, TP), 0)
        row_h = jax.lax.broadcasted_iota(i32, (HP, TP), 0)

        def ln_tile(j):
            xc = xt_s[:, j * HT:(j + 1) * HT]
            xn1_s[:, j * HT:(j + 1) * HT] = _pack(_layernorm_t(xc.astype(f32)).astype(bf16))

        def h_tile(j, r0=0, r1=D):
            xn = _unpack(xn1_s[:, j * HT:(j + 1) * HT])
            ht_s[j + 1, r0 // 2:r1 // 2, :] = _pack(
                _gelu(_dot(_unpack(w1T_s[r0 // 2:r1 // 2]), xn)).astype(bf16))

        def kb_pieces(p_lo, p_hi):
            for p in range(p_lo, p_hi):
                g, d0 = divmod(p * 8, G)
                kp = k_s[g, 0:NOFF // 2, :]
                cols = jnp.concatenate(
                    [jnp.broadcast_to(kp[:, d:d + 1], (NOFF // 2, 128))
                     for d in range(d0, d0 + 8)], axis=0)
                kb_s[p * 8:(p + 1) * 8] = _unpack(cols).astype(f32).reshape(8, NOFF, 128)

        def k_part(t0, rk):
            n = rk.shape[1]
            ones_row = jnp.where(jax.lax.broadcasted_iota(i32, (16, n), 0) == 0, 1.0, 0.0)
            for g in range(4):
                kt = jnp.concatenate([rk[g * G:(g + 1) * G, :], ones_row], axis=0)
                k_s[g, t0 // 2:(t0 + n) // 2, :] = _pack(kt.astype(bf16).T)

        def k_only(t0, t1):
            k_part(t0, _dot(_unpack(wqkvT_s[D // 2:D]), xt_s[:, t0:t1]))

        def qkv_chunk(c, with_k=True):
            t0 = c * TP
            xc = xt_s[:, t0:t0 + TP]
            if with_k:
                r = _dot(_unpack(wqkvT_s[...]), xc)
                k_part(t0, r[D:2 * D])
                rv = r[2 * D:]
            else:
                lhs = jnp.concatenate([wqkvT_s[0:D // 2], wqkvT_s[D:]], axis=0)
                r = _dot(_unpack(lhs), xc)
                rv = r[D:]
            qf = r[0:D, :] * QSCALE
            for v in range(NV):
                g, odd = divmod(v, 2)
                lo = (G - SL) * odd
                qg = qf[g * G + lo:g * G + lo + SL, :]
                for j in range(HV):
                    h0 = (odd * HV + j) * DH - lo
                    qm = jnp.where((row_s >= h0) & (row_s < h0 + DH), qg, 0.0)
                    for b in range(TP // TQ):
                        qp_s[t0 // TQ + b, v, :, j * TQ:(j + 1) * TQ] = _pack(
                            qm[:, b * TQ:(b + 1) * TQ].astype(bf16))
            for tl in range(TP // 128):
                if t0 // 128 + tl >= NT:
                    qf_s[t0 // 128 + tl, 0:D, :] = qf[:, tl * 128:(tl + 1) * 128]
            for h in range(H):
                vh = rv[h * DH:h * DH + HP, :]
                vh = jnp.where(row_h < DH, vh, jnp.where(row_h == DH, 1.0, 0.0))
                vt_s[h, :, t0:t0 + TP] = _pack(vh.astype(bf16))
            g_s[:, t0:t0 + TP] = jax.nn.sigmoid(rv[D:D + 1, :])
            if c in QCC:
                for i in range(56):
                    r8, tl = QCC.index(c) * 28 + i // 2, i % 2
                    rr = (i % 14) * 96
                    dep = r[rr:rr + 8, (i // 14) * 128:(i // 14 + 1) * 128]
                    fill_qc(1, r8, tl, dep)

        n0, na, nb, nt = X0T // HT, XA // HT, XB // HT, T // HT
        cp_x0.wait()
        for j in range(n0):
            ln_tile(j)
        cp_w1a.wait()
        cp_xb.start()
        w1T_s[0:W1A // 2] = _pack(w1_v[:, 0:W1A].T)
        for j in range(n0 - 1):
            h_tile(j, 0, W1A)
        cp_w1b.wait()
        cp_xa.wait()
        cp_xc.start()
        cp_wqkv.start()
        cp_gw.start()
        h_tile(n0 - 1, 0, W1A)
        w1T_s[W1A // 2:] = _pack(w1_v[:, W1A:].T)
        for j in range(n0, na):
            ln_tile(j)
        for j in range(n0):
            h_tile(j, W1A, D)
        for j in range(n0, na - 1):
            h_tile(j)
        cp_xb.wait()
        cp_w3.start()
        cp_w2.start()
        cp_wo.start()
        cp_w4.start()
        for j in range(na, nb):
            ln_tile(j)
        for j in range(na - 1, nb - 1):
            h_tile(j)
        cp_xc.wait()
        cp_wqkv.wait()
        cp_gw.wait()
        row16 = jax.lax.broadcasted_iota(i32, (16, D), 0)
        gw = jnp.broadcast_to(gw_v[...].astype(f32).reshape(1, D), (16, D))
        wqkvT_s[GROW // 2:GROW // 2 + 8, :] = _pack(jnp.where(row16 == 0, gw, 0.0).astype(bf16))
        wqkvT_s[0:GROW // 2, :] = _pack(wqkv_v[...].T)
        for j in range(nb, nt):
            ln_tile(j)
        for j in range(nb - 1, nt - HLATE):
            h_tile(j)
        k_only(0, NOFF)
        kb_pieces(0, KB0)
        for j in range(nt - HLATE, nt):
            h_tile(j)
        k_only(NOFF, TP)
        qkv_chunk(0, with_k=False)
        cp_w3.wait()
        cp_w2.wait()
        cp_wo.wait()
        cp_w4.wait()
        kb_pieces(KB0, D // 8)
        qkv_chunk(1)
        qkv_chunk(2)
        w3T_s[...] = _pack(w3_v[...].T)
        qkv_chunk(3)
        zlast = jnp.zeros((16, W), bf16)
        for v in range(NV):
            sv0 = _dot(_unpack(k_s[v // 2, 0:NOFF // 2, :]),
                       qk_rhs(v, _unpack(qp_s[0, v]), zlast))
            sv_s[v] = sv0
            mx_s[v] = jnp.max(sv0[0:MB * XK].reshape(MB * XK // 8, 8, W), axis=0)
        qs_s[...] = qp_s[0]
        for r8 in range(D // 16):
            fill_hs(0, r8, None)
        w2T_s[...] = _pack(w2_v[...].T)
        wo32 = wo_v[...].astype(f32)
        zrows = jnp.zeros((HP - DH, D), f32)
        parts = []
        for h in range(H):
            parts.append(wo32[h * DH:(h + 1) * DH, :])
            parts.append(zrows)
        woT_s[...] = _pack(jnp.concatenate(parts, axis=0).T.astype(bf16))

    q0 = pl.multiple_of(step * TQ, TQ)
    gate = g_s[:, pl.ds(q0, TQ)]
    st = {}
    total = NV * NU
    nw4 = F // KC
    w3_at = total - W3_BACK

    def x_block(v, j, tl, b, deps):
        h = v * HV + j
        feat = slice(h * DH, (h + 1) * DH)
        q = qc_s[tl, feat].reshape(DH // XP, XP, 8, 128)
        q0_ = _after(q[:, 0:1], jnp.stack(deps)[:, None])
        q = jnp.concatenate([q0_, q[:, 1:]], axis=1).reshape(DH, 1, 8, 128)
        kb = kb_s[feat, b * XK:(b + 1) * XK, :].reshape(DH, XK // 8, 8, 128)
        sx = jnp.sum(kb * q, axis=0)
        c0 = j * TQ + tl * 128
        sv_s[v, b * XK:(b + 1) * XK, c0:c0 + 128] = sx.reshape(XK, 128)
        if b < MB:
            mx = jnp.max(sx, axis=0)
            st['xmx'] = mx if b == 0 else jnp.maximum(st['xmx'], mx)
        if b == MB - 1:
            mx_s[v, :, c0:c0 + 128] = st['xmx']

    xlist = [(v, j, tl, b) for v in range(NV) for j in range(HV) for tl in range(NT)
             for b in range(NOFF // XK)]
    npieces = len(xlist) * (DH // XP)
    wslot = [0 if w3_at - NPAUSE <= t < w3_at else WSL[t % NU] for t in range(total)]
    ngate = (sum(wslot) * (CK // GR) + NT * WT3 * (F // GR)
             + ((nw4 - 1) * WT4 + NT * WT2 + WTE) * (D // GR))
    xstate = dict(done=0, gate=0, started=-1, n=0, credit=0.0)
    xdeps = []
    nxt1 = jnp.minimum(step + 1, NSTEP - 1)
    nxt2 = jnp.minimum(step + 2, NSTEP - 1)
    qtasks = []

    def side_work(res, weight):
        for r_ in range(0, res.shape[0], GR):
            fire = False
            if xlist and weight and xlist[0][0] <= xstate['started']:
                left = npieces - xstate['done'] - xstate['credit']
                xstate['credit'] += weight * left / max(ngate - xstate['gate'] - 20, weight)
                fire = xstate['credit'] >= 1.0 - 1e-9
            xstate['gate'] += weight
            if fire:
                xstate['credit'] -= 1.0
                xstate['done'] += 1
                xdeps.append(res[r_:r_ + 8, 0:128])
                if len(xdeps) == DH // XP:
                    xb = xlist.pop(0)
                    x_block(*xb, list(xdeps))
                    xdeps.clear()
                    if not xlist or xlist[0][0] != xb[0]:
                        qtasks.extend(functools.partial(fill_qc, nxt2, r8, tl)
                                      for r8 in range(xb[0] * 7, (xb[0] + 1) * 7)
                                      for tl in range(NT))
            xstate['n'] += 1
            if qtasks and xstate['n'] % (QEVERY if xlist else 3) == 0:
                qtasks.pop(0)(res[r_:r_ + 8, 0:128])

    def b_part1():
        x = xt_s[:, pl.ds(q0, TQ)].astype(f32)
        zs = [_dot(_unpack(w2T_s[...]), _unpack(hs_s[:, tl * 128:(tl + 1) * 128]))
              for tl in range(NT)]
        for z in zs:
            side_work(z, WT2)
        x1 = x + jnp.concatenate(zs, axis=1)
        y_s[...] = x1
        xn_s[...] = _pack(_layernorm_t(x1).astype(bf16))
        qtasks.extend(functools.partial(fill_hs, nxt1, r8) for r8 in range(D // 16))

    def b_w3(i, tl):
        rows = slice(i * KC // 2, (i + 1) * KC // 2)
        z = _dot(_unpack(w3T_s[rows]), _unpack(xn_s[:, tl * 128:(tl + 1) * 128]))
        h2_s[rows, tl * 128:(tl + 1) * 128] = _pack(_gelu(z).astype(bf16))
        side_work(z, WT3)

    def b_w4(i, wt):
        yi = y_s[...] + _dot(w4t_s[:, i * KC:(i + 1) * KC],
                             _unpack(h2_s[i * KC // 2:(i + 1) * KC // 2, :]))
        y_s[...] = yi
        side_work(yi, wt)

    def b_mlp():
        for i in range(nw4):
            for tl in range(NT):
                b_w3(i, tl)
            if i > 0:
                b_w4(i - 1, WT4)

    def b_wo_a():
        a_ = _dot(_unpack(woT_s[:, 0:HK]), _unpack(ot_s[0:H // 2].reshape(HK // 2, TQ)))
        st['a'] = gate * a_
        side_work(a_, WTE)

    extra = {0: b_part1, w3_at: b_mlp, total: b_wo_a,
             total + 1: functools.partial(b_w4, nw4 - 1, 0)}

    row16w = jax.lax.broadcasted_iota(i32, (16, W), 0)
    rhs, svm, ptile, acc = {}, {}, {}, {}
    amax = lmin = None

    def probs(s):
        return [jnp.exp2(s[:, j * TQ:(j + 1) * TQ]).astype(bf16) for j in range(HV)]

    def pv(v, kt, ps):
        oc = [_dot(_unpack(vt_s[v * HV + j, :, kt * CK:(kt + 1) * CK]), ps[j])
              for j in range(HV)]
        acc[v] = [a_ + o_ for a_, o_ in zip(acc[v], oc)] if v in acc else oc
        return oc

    for t in range(total + 2):
        if t < total and t % NU == 0:
            v = t // NU
            m0 = jnp.max(mx_s[v], axis=0, keepdims=True).astype(bf16).astype(f32)
            last = jnp.where(row16w == 0, -m0, 0.0).astype(bf16)
            rhs[v] = qk_rhs(v, _unpack(qs_s[v]), last)
            svm[v] = sv_s[v] - m0
            xstate['started'] = v
        if t in extra:
            extra[t]()
        if t < total:
            v, c = divmod(t, NU)
            kt = NVT + c
            kp = k_s[v // 2, kt * CK // 2:(kt + 1) * CK // 2, :]
            kp = jnp.concatenate([kp[i * 8:(i + 1) * 8] for i in reversed(range(8))], axis=0)
            sr = _dot(_unpack(kp), rhs[v])
            ptile[t] = probs(jnp.concatenate(
                [sr[i * 16:(i + 1) * 16] for i in reversed(range(8))], axis=0))
            if c == NU - 1:
                qtasks[0:0] = [functools.partial(fill_qs, nxt1, v, p_) for p_ in range(SL // 16)]
            side_work(sr, wslot[t])
            if c in FPOS:
                vt_ = FPOS.index(c)
                pv(v, vt_, probs(svm[v][vt_ * CK:(vt_ + 1) * CK]))
        if 1 <= t <= total:
            v, c = divmod(t - 1, NU)
            oc = pv(v, NVT + c, ptile[t - 1])
            if c == NU - 1:
                for j in range(HV):
                    l = acc[v][j][DH:DH + 1, :]
                    am = jnp.max(jnp.abs(acc[v][j]).reshape(HP // 8, 8, TQ), axis=0)
                    amax = am if amax is None else jnp.maximum(amax, am)
                    lmin = l if lmin is None else jnp.minimum(lmin, l)
                    ot_s[v * HV + j] = _pack((acc[v][j] * (1.0 / l)).astype(bf16))
    while qtasks:
        qtasks.pop(0)(oc[0][0:8, 0:128])
    assert not xlist

    rest = st['a'] + (1.0 - gate) * y_s[...]
    a = _dot(_unpack(woT_s[:, HK:]), _unpack(ot_s[H // 2:].reshape(HK // 2, TQ)))
    out_ref[...] = (gate * a + rest).astype(out_ref.dtype)

    safe = jnp.where((amax < L_HI) & (lmin > L_LO), 1.0, 0.0)
    unsafe = jnp.min(safe) < 0.5

    @pl.when(unsafe)
    def _fallback():
        def head_pair(v, carry):
            fr_s[...] = jnp.zeros((CK // 2, W), u32)
            off = pl.multiple_of((v % 2) * ((G - SL) // 2), 8)
            fr_s[pl.ds(off, SL // 2), :] = qp_s[step, v]

            def scores(c, m):
                rk = pl.ds(pl.multiple_of(c * (CK // 2), CK // 2), CK // 2)
                s = _dot(_unpack(k_s[v // 2, rk, :]), _unpack(fr_s[...]))
                fs_s[pl.ds(pl.multiple_of(c * CK, CK), CK), :] = s
                return jnp.maximum(m, jnp.max(s, axis=0, keepdims=True))

            m = jax.lax.fori_loop(0, NC, scores, jnp.full((1, W), -jnp.inf, f32))

            def values(c, o):
                r0 = pl.multiple_of(c * CK, CK)
                p = jnp.exp2(fs_s[pl.ds(r0, CK), :] - m)
                return tuple(
                    o[j] + _dot(_unpack(vt_s[v * HV + j, :, pl.ds(r0, CK)]),
                                p[:, j * TQ:(j + 1) * TQ].astype(bf16))
                    for j in range(HV))

            o = jax.lax.fori_loop(0, NC, values,
                                  tuple(jnp.zeros((HP, TQ), f32) for _ in range(HV)))
            for j in range(HV):
                ot_s[v * HV + j] = _pack((o[j] * (1.0 / o[j][DH:DH + 1, :])).astype(bf16))
            return carry

        jax.lax.fori_loop(0, NV, head_pair, 0)
        a2 = _dot(_unpack(woT_s[...]), _unpack(ot_s[...].reshape(HK, TQ)))
        out_ref[...] = (gate * a2 + (1.0 - gate) * y_s[...]).astype(out_ref.dtype)


@jax.jit
def pallas_gated_mix__mha_block__mixer_s_mlp__prompt_kernel(
    A_x: jax.Array,
    A_wqkv: jax.Array,
    A_wo: jax.Array,
    B_x: jax.Array,
    B_w1: jax.Array,
    B_w2: jax.Array,
    B_w3: jax.Array,
    B_w4: jax.Array,
    gate_w: jax.Array,
):
    xt = A_x.reshape(T, D).T
    w4t = B_w4.T
    hbm = pl.BlockSpec(memory_space=pltpu.MemorySpace.HBM)

    out_t = pl.pallas_call(
        _kernel,
        grid=(NSTEP,),
        in_specs=[hbm] * 8,
        out_specs=pl.BlockSpec((D, TQ), lambda i: (0, i)),
        out_shape=jax.ShapeDtypeStruct((D, T), bf16),
        scratch_shapes=[
            pltpu.VMEM((D, T), bf16),
            pltpu.VMEM((D, 3 * D), bf16),
            pltpu.VMEM((D, D), bf16),
            pltpu.VMEM((D, D), bf16),
            pltpu.VMEM((D, D), bf16),
            pltpu.VMEM((D, F), bf16),
            pltpu.VMEM((D, F), bf16),
            pltpu.VMEM((D,), bf16),
            pltpu.SemaphoreType.DMA((12,)),
            pltpu.VMEM((GROW // 2 + 8, D), u32),
            pltpu.VMEM((D // 2, D), u32),
            pltpu.VMEM((D // 2, D), u32),
            pltpu.VMEM((F // 2, D), u32),
            pltpu.VMEM((D // 2, H * HP), u32),
            pltpu.VMEM((4, T // 2, 128), u32),
            pltpu.VMEM((NSTEP, NV, SL // 2, W), u32),
            pltpu.VMEM((H, HP // 2, T), u32),
            pltpu.VMEM((T // HT + 2, 256, HT), u32),
            pltpu.VMEM((1, T), f32),
            pltpu.VMEM((H, HP // 2, TQ), u32),
            pltpu.VMEM((D, TQ), f32),
            pltpu.VMEM((D // 2, TQ), u32),
            pltpu.VMEM((F // 2, TQ), u32),
            pltpu.VMEM((D // 2, T), u32),
            pltpu.VMEM((T // 128, 512, 128), f32),
            pltpu.VMEM((D, NOFF, 128), f32),
            pltpu.VMEM((NV, NOFF, W), f32),
            pltpu.VMEM((NT, D, 8, 128), f32),
            pltpu.VMEM((NV, SL // 2, W), u32),
            pltpu.VMEM((T, W), f32),
            pltpu.VMEM((CK // 2, W), u32),
            pltpu.VMEM((D // 2, TQ), u32),
            pltpu.VMEM((NV, 8, W), f32),
        ],
        compiler_params=pltpu.CompilerParams(
            dimension_semantics=("arbitrary",),
            vmem_limit_bytes=120 * 1024 * 1024,
        ),
        name="gated_mix",
    )(xt, A_wqkv, A_wo, B_w1, B_w2, B_w3, w4t, gate_w)
    return out_t.T.reshape(1, T, D)
```
